```python
import os as _os
_os.environ.setdefault("JAX_PLATFORMS", "cpu")
import jax
import jax.numpy as jnp

def _softmax(x, axis=-1):
    return jax.nn.softmax(x, axis=axis)
def _gelu(x):
    return jax.nn.gelu(x, approximate=True)
def _silu(x):
    return jax.nn.silu(x)
def _sigmoid(x):
    return jax.nn.sigmoid(x)
def _layernorm(x, axis=-1, eps=1e-5):
    m = jnp.mean(x, axis=axis, keepdims=True)
    v = jnp.var(x, axis=axis, keepdims=True)
    return (x - m) / jnp.sqrt(v + eps)
def _scatter_add(tgt, idx, src, axis=0):
    return tgt.at[idx].add(src)
def _segment_sum(src, seg, n):
    return jax.ops.segment_sum(src, seg, n)
class _Rng:
    def __init__(self, key):
        self._k = key
    def _next(self):
        self._k, sub = jax.random.split(self._k)
        return sub
    def normal(self, shape):
        return jax.random.normal(self._next(), shape, dtype=jnp.bfloat16)
    def randint(self, lo, hi, shape):
        return jax.random.randint(self._next(), shape, lo, hi, dtype=jnp.int32)
    def uniform(self, shape, lo=0.0, hi=1.0):
        return jax.random.uniform(self._next(), shape, jnp.bfloat16, lo, hi)
    def permutation(self, n):
        return jax.random.permutation(self._next(), n)


kernel_name = 'interleave_layers__sliding_block_cached__mixer_channel_mlp__decode'

def setup_inputs():
    _rng = _Rng(jax.random.key(int.from_bytes(__import__("os").urandom(4), "little")))
    _w = (lambda a: (lambda t: t.astype(jnp.bfloat16) if jnp.issubdtype(t.dtype, jnp.floating) else t)(jnp.asarray(a)))
    def _A_setup():
        B, Sq, D = 8, 1, 640
        Hq, Hkv, Sk, Dh = 32, 32, 4096, 128
        assert Hq % Hkv == 0, (Hq, Hkv)
        return {
            "x": _w((lambda *s: _rng.normal(s) * 0.05)(B, Sq, D)),
            "k_cache": _w((lambda *s: _rng.normal(s) * 1.6)(B, Hkv, Sk, Dh)),
            "v_cache": _w((lambda *s: _rng.normal(s) * 0.8)(B, Hkv, Sk, Dh)),
            "wq": _w((lambda *s: _rng.normal(s) * 1.6)(D, Hq * Dh) * (D ** -0.5)),
            "wo": _w((lambda *s: _rng.normal(s) * 0.8)(Hq * Dh, D) * ((Hq * Dh) ** -0.5)),
        }
    _A_in = _A_setup()

    def _B_setup():
        B, S, D, F = 8, 1, 640, 1728
        return {
            "x": _w((lambda *s: _rng.normal(s) * 0.05)(B, S, D)),
            "w1": _w((lambda *s: _rng.normal(s) * 0.4)(D, F) * (D ** -0.5)),
            "b1": _w((lambda *s: _rng.normal(s) * 0.4)(F)),
            "w2": _w((lambda *s: _rng.normal(s) * 0.4)(F, D) * (F ** -0.5)),
            "b2": _w((lambda *s: _rng.normal(s) * 0.2)(D)),
        }
    _B_in = _B_setup()

    return {
        "A_x": _A_in["x"],
        "A_k_cache": _A_in["k_cache"],
        "A_v_cache": _A_in["v_cache"],
        "A_wq": _A_in["wq"],
        "A_wo": _A_in["wo"],
        "B_x": _B_in["x"],
        "B_w1": _B_in["w1"],
        "B_b1": _B_in["b1"],
        "B_w2": _B_in["w2"],
        "B_b2": _B_in["b2"],
    }

def reference(A_x, A_k_cache, A_v_cache, A_wq, A_wo, B_x, B_w1, B_b1, B_w2, B_b2):
    def _A_ref(x, k_cache, v_cache, wq, wo):
        B, Sq, D = x.shape
        Hq, Dh = 32, 128
        Hkv, Sk = k_cache.shape[1], k_cache.shape[2]
        W = min(4096, max(256, Sk // 4))
        rep = Hq // Hkv
        q = (lambda x, *d: x.transpose(*d))((x @ wq).reshape(B, Sq, Hq, Dh), 0, 2, 1, 3)
        k = jnp.repeat(k_cache[:, :, Sk - W:, :], rep, axis=1)
        v = jnp.repeat(v_cache[:, :, Sk - W:, :], rep, axis=1)
        scores = jnp.einsum("bhqd,bhkd->bhqk", q, k) * (Dh ** -0.5)
        p = _softmax(scores, axis=-1)
        o = jnp.einsum("bhqk,bhkd->bhqd", p, v)
        return (lambda x, *d: x.transpose(*d))(o, 0, 2, 1, 3).reshape(B, Sq, Hq * Dh) @ wo

    def _B_ref(x, w1, b1, w2, b2):
        y = _layernorm(x, axis=-1)
        h = _gelu(jnp.einsum("bsd,df->bsf", y, w1) + b1)
        return jnp.einsum("bsf,fd->bsd", h, w2) + b2

    x = A_x
    x = x + _A_ref(_layernorm(x, axis=-1), A_k_cache, A_v_cache, A_wq, A_wo)
    x = x + _B_ref(_layernorm(x, axis=-1), B_w1, B_b1, B_w2, B_b2)
    x = x + _A_ref(_layernorm(x, axis=-1), A_k_cache, A_v_cache, A_wq, A_wo)
    x = x + _B_ref(_layernorm(x, axis=-1), B_w1, B_b1, B_w2, B_b2)
    return x
```

```python
import jax
import jax.numpy as jnp
from jax import lax
import jax.experimental.pallas as pl
import jax.experimental.pallas.tpu as pltpu

B, D, H, DH, SK, F = 8, 640, 32, 128, 4096, 1728
W = min(4096, max(256, SK // 4))
G = 8
NG = H // G
CH = 128
NR = W // CH
ND = D // 128
UB = NG * NR
ORDER = (0, 4, 2, 6, 1, 5, 3, 7)
EPS = 1e-5
QSCALE = DH ** -0.5 * 1.4426950408889634
F32, BF16, U32 = jnp.float32, jnp.bfloat16, jnp.uint32

MLP_G, MLP_LAG = 2, 3
FM = 1152
STR = 10
LAG_S, LAG_E, LAG_F = 2, 3, 5
FGROUPS = (4,) * 7 + (2, 1, 1)
MXU_HEADS = (1, 2)
LC, LD = 2, 0
ONLYTAIL = False
FUSE = 0
AHEAD = 3
P0 = 2
SCOPES = False
NOCOMP = 0
STOP = 0
SEMCHK = False
RS = 6
VQ = (0, 1)
TS = (5, 7, 8)
VISS = (10, 32, 52)


class _scope:
    def __init__(self, name):
        self.cm = jax.named_scope(name) if (SCOPES is True or (SCOPES and name in SCOPES)) else None

    def __enter__(self):
        if self.cm is not None:
            self.cm.__enter__()

    def __exit__(self, *a):
        if self.cm is not None:
            self.cm.__exit__(*a)


def _bf16(u):
    return pltpu.bitcast(u, BF16)


def _dot(a, b, transposed=False):
    return lax.dot_general(a, b, (((1,), (1 if transposed else 0,)), ((), ())),
                           preferred_element_type=F32)


def _cols(x, n):
    return [x[:, j * 128:(j + 1) * 128] for j in range(n)]


def _hint(i, n):
    return i if isinstance(i, int) else pl.multiple_of(i, n)


def _rstd(x):
    c = x - jnp.mean(x, axis=-1, keepdims=True)
    v = jnp.mean(c * c, axis=-1, keepdims=True)
    return c, v, lax.rsqrt(v + EPS)


def _kernel(x_hbm, k_hbm, v_hbm, wq_hbm, wo_hbm, w1t_hbm, b1_hbm, w2_hbm, b2_hbm,
            o_ref,
            x_s, b1_s, b2_s, wq_s, wo_s, w1t_s, w2_s,
            xf, bias1, cs1, bias1c, bias2, wq_p, wo_p, w1_p, w2_p, wqt, w1tc, w2h,
            kbuf, vbuf, kt, ktb, csq, tr, q_all, p_last, l_last, outf, wsem, kvsem, lsem):
    FV = F - FM
    k32 = k_hbm.bitcast(U32)
    v32 = v_hbm.bitcast(U32)
    row = lax.broadcasted_iota(jnp.int32, (8, 128), 0)

    small = [pltpu.make_async_copy(x_hbm, x_s, wsem.at[0]),
             pltpu.make_async_copy(b1_hbm, b1_s, wsem.at[0]),
             pltpu.make_async_copy(b2_hbm, b2_s, wsem.at[0])]

    def issue_qo(lo, hi):
        def body(i, _):
            for u in range(5):
                r = pl.ds(pl.multiple_of((u * 16 + (i >> 1)) * 8, 8), 8)
                c = pl.ds(pl.multiple_of((i & 1) * 2048, 2048), 2048)
                pltpu.make_async_copy(wq_hbm.at[r, c], wq_s.at[r, c], wsem.at[0]).start(priority=0)
                if u < 4:
                    r = pl.ds(pl.multiple_of((u * 32 + i) * 32, 32), 32)
                    pltpu.make_async_copy(wo_hbm.at[r], wo_s.at[r], wsem.at[0]).start(priority=1)
        lax.fori_loop(lo, hi, body, None)

    def issue_mlp(lo, hi):
        def body(i, _):
            for u in range(2):
                r = pl.ds(pl.multiple_of((u * 27 + i) * 32, 32), 32)
                pltpu.make_async_copy(w1t_hbm.at[r], w1t_s.at[r], wsem.at[1]).start(priority=0)
                pltpu.make_async_copy(w2_hbm.at[r], w2_s.at[r], wsem.at[1]).start(priority=1)
        lax.fori_loop(lo, hi, body, None)

    def chunk(src, dst, b, h, r, sem):
        r0 = _hint(r * (CH // 2), CH // 2)
        return pltpu.make_async_copy(src.at[b, h, pl.ds((SK - W) // 2 + r0, CH // 2)],
                                     dst.at[b & 1, h, pl.ds(r0, CH // 2)], sem)

    h2, h3 = H - 2 * G, H - G
    u_keys, u_last = B * UB - 2 * NR, B * UB - NR
    sem_v2, sem_piece = wsem.at[0], [wsem.at[1], lsem.at[0], lsem.at[1], lsem.at[2]]

    def issue_kv(lo, hi):
        def body(u, _):
            b = u >> 5
            g = (u >> 3) & (NG - 1)
            r = ((u & 1) << 2) | (u & 2) | ((u >> 2) & 1)

            @pl.when(u < u_keys)
            def _():
                for i in ORDER:
                    chunk(k32, kbuf, b, g * G + i, r, kvsem.at[g]).start(priority=0)
                    chunk(v32, vbuf, b, g * G + i, r, kvsem.at[g]).start(priority=1)

            @pl.when(u >= u_keys)
            def _():
                for i in ORDER:
                    chunk(k32, kbuf, B - 1, h2 + i, r, kvsem.at[NG - 2]).start(priority=0)
                    if i < G // 2:
                        c = chunk(k32, kbuf, B - 1, h3 + G // 2 + i, r, kvsem.at[NG - 1])
                    else:
                        c = chunk(v32, vbuf, B - 1, h2 + i, r, sem_v2)
                    c.start(priority=1)
        lax.fori_loop(jnp.minimum(lo, u_last), jnp.minimum(hi, u_last), body, None)

    def wait_all(ref, sem):
        pltpu.make_async_copy(ref, ref, sem).wait()

    issue_qo(0, 1)
    for c in small:
        c.start()
    issue_qo(1, 32)
    issue_mlp(0, F // 64)
    issue_kv(0, P0)
    for c in small:
        c.wait()
    wait_all(wq_s, wsem.at[0])
    wait_all(wo_s, wsem.at[0])

    xf[...] = x_s[...].astype(F32)
    b1 = b1_s[...].astype(F32).reshape(1, F)
    bias1[...] = jnp.broadcast_to(b1[:, :FM], (8, FM))
    b1v = jnp.concatenate([b1[:, FM:], jnp.zeros((1, -FV % 128), F32)], axis=1)
    for n in range(0, FV, 128):
        t = jnp.broadcast_to(b1v[:, n:n + 128], (128, 128)).T
        bias1c[n:min(n + 128, FV)] = t[:min(128, FV - n)]
    bias2[...] = jnp.broadcast_to(b2_s[...].astype(F32).reshape(1, D), (8, D))
    c, _, r = _rstd(xf[...])
    y_all = (c * r).astype(BF16)

    @pl.loop(0, NG)
    def _(g):
        with _scope("prep_wq"):
            for i in range(G):
                h = g * G + i
                w = wq_s[:, pl.ds(pl.multiple_of(h * DH, DH), DH)]
                wq_p[h] = pltpu.bitcast(w, U32)
                q_all[pl.ds(h, B, stride=H), :] = QSCALE * jnp.dot(
                    y_all, w, preferred_element_type=F32)
                w = w.T.astype(F32)
                wqt[h] = (w - jnp.mean(w, axis=1, keepdims=True)) * QSCALE

        issue_kv(P0 + 2 * g, P0 + 2 * g + 2)

    for i, h in enumerate(MXU_HEADS):
        csq[i] = jnp.broadcast_to(
            jnp.sum(wq_s[:, h * DH:(h + 1) * DH].astype(F32), axis=0, keepdims=True), (8, 128))

    with _scope("prep_wo"):
        @pl.loop(0, H)
        def _(h):
            r = pl.ds(pl.multiple_of(h * DH, DH), DH)
            for j in range(ND):
                wo_p[j, pl.ds(pl.multiple_of(h * (DH // 2), DH // 2), DH // 2)] = pltpu.bitcast(
                    wo_s[r, j * 128:(j + 1) * 128], U32)

    issue_kv(P0 + 8, P0 + 10)
    wait_all(w1t_s, wsem.at[1])
    wait_all(w2_s, wsem.at[1])
    with _scope("prep_w1"):
        for n in range(FM // 128):
            t = w1t_s[n * 128:(n + 1) * 128, :].T
            w1_p[n] = pltpu.bitcast(t, U32)
            cs1[n] = jnp.broadcast_to(jnp.sum(t.astype(F32), axis=0, keepdims=True), (8, 128))
        t = w1t_s[FM:F, :].astype(F32)
        w1tc[...] = t - jnp.mean(t, axis=1, keepdims=True)

    issue_kv(P0 + 10, P0 + 12)
    with _scope("prep_w2"):
        for j in range(ND):
            w = 0.5 * w2_s[0:FM, j * 128:(j + 1) * 128].astype(F32)
            w2_p[j] = pltpu.bitcast(w.astype(BF16), U32)
        w2h[...] = 0.5 * w2_s[FM:F, :].astype(F32)

    issue_kv(P0 + 12, 20 + AHEAD)

    def scores(b, h0):
        q = q_all[pl.ds(_hint(b * H + h0, G), G), :]
        s = None
        for i in range(G):
            si = _cols(_dot(q, _bf16(kbuf[b & 1, h0 + i]), transposed=True), NR)
            s = si if s is None else [jnp.where(row == i, a, c) for a, c in zip(si, s)]
        s = jnp.concatenate(s, axis=1)
        p = jnp.exp2(s - jnp.max(s, axis=-1, keepdims=True))
        return p, jnp.sum(p, axis=-1, keepdims=True)

    def weighted_values(p, b, h0, heads):
        o = None
        for i in heads:
            oi = _dot(p, _bf16(vbuf[b & 1, h0 + i]))
            o = oi if o is None else jnp.where(row == i, oi, o)
        return o

    def project(o, h0, heads):
        lhs = jnp.concatenate([jnp.where(row == i, o, 0.0) for i in heads], axis=1)
        r0 = pl.ds(_hint((h0 + heads[0]) * (DH // 2), DH // 2), len(heads) * DH // 2)
        w = jnp.concatenate([_bf16(wo_p[j, r0]) for j in range(ND)], axis=1)
        return _dot(lhs, w)

    def attn_group(b, g):
        if NOCOMP:
            if NOCOMP == 1: pl.delay(1550)
            return jnp.zeros((8, D), F32)
        p, l = scores(b, g * G)
        o = weighted_values(p, b, g * G, range(G))
        return project(o / l, g * G, range(G))

    def row_sum(acc):
        return jnp.broadcast_to(jnp.sum(acc, axis=0, keepdims=True), acc.shape)

    def gelu2(a):
        c = 0.7978845608028654
        return a + a * jnp.tanh(a * (c + (c * 0.044715) * (a * a)))

    def mlp(x):
        if NOCOMP:
            if NOCOMP == 1: pl.delay(600)
            return x
        xr = x.astype(BF16).astype(F32)
        mean = jnp.mean(xr, axis=-1, keepdims=True)
        c = xr - mean
        v = jnp.mean(c * c, axis=-1, keepdims=True)
        r1 = lax.rsqrt(v + EPS)
        rs = jnp.broadcast_to(r1 * lax.rsqrt(v * r1 * r1 + EPS), (8, 128))
        mrs = jnp.broadcast_to(mean, (8, 128)) * rs

        def first(ns):
            w = jnp.concatenate([_bf16(w1_p[n]) for n in ns], axis=1)
            a = _cols(_dot(xr, w), len(ns))
            return [gelu2(t * rs + (bias1[:, n * 128:(n + 1) * 128] - mrs * cs1[n]))
                    for t, n in zip(a, ns)]

        def second(ns, hid):
            w = jnp.concatenate([_bf16(w2_p[j, ns[0] * 64:(ns[-1] + 1) * 64]) for j in range(ND)],
                                axis=1)
            return _dot(jnp.concatenate(hid, axis=1), w)

        groups = [range(n, min(n + MLP_G, FM // 128)) for n in range(0, FM // 128, MLP_G)]
        hid, out = [], None
        for t in range(len(groups) + MLP_LAG):
            if t < len(groups):
                hid.append(first(groups[t]))
            if t >= MLP_LAG:
                u = second(groups[t - MLP_LAG], hid[t - MLP_LAG])
                out = u if out is None else out + u
        xc = _cols(xr, ND)
        acc = [None] * ND
        for i in range(0, FV, 8):
            t = [w1tc[i:i + 8, j * 128:(j + 1) * 128] * xc[j] for j in range(ND)]
            t = (t[0] + t[1]) + (t[2] + t[3]) + t[4]
            t = jnp.broadcast_to(jnp.sum(t, axis=1, keepdims=True), (8, 128))
            hv = gelu2(t * rs + bias1c[i:i + 8])
            for j in range(ND):
                u = w2h[i:i + 8, j * 128:(j + 1) * 128] * hv
                acc[j] = u if acc[j] is None else acc[j] + u
        return (x + bias2[...]) + row_sum(jnp.concatenate(acc, axis=1)) + out

    def batch_row(b, done):
        base = b * UB + AHEAD

        def layer(l, x):
            @pl.when(l == 1)
            def _():
                issue_kv(base + 39, base + 40)
                with _scope("q2"):
                    c, _, r = _rstd(x)
                    y = c * r
                    for g in range(NG):
                        w = jnp.concatenate([_bf16(wq_p[g * G + i]) for i in range(G)], axis=1)
                        qr = _cols(_dot(y, w), G)
                        q = qr[0]
                        for i in range(1, G):
                            q = jnp.where(row == i, qr[i], q)
                        q_all[pl.ds(pl.multiple_of(b * H + g * G, G), G), :] = q * QSCALE

            def group(g, acc):
                lo = jnp.where(l == 0, 20 + 3 * g, jnp.where(g == 0, 40, 38 + 3 * g))
                hi = jnp.where(l == 0, jnp.where(g == NG - 1, 36, 23 + 3 * g), 41 + 3 * g)
                with _scope("iss"):
                    issue_kv(base + lo, base + hi)

                @pl.when(l == 0)
                def _():
                    hs = pl.ds(g * G, G)
                    wait_all(kbuf.at[b & 1, hs], kvsem.at[g])
                    wait_all(vbuf.at[b & 1, hs], kvsem.at[g])

                with _scope("att"):
                    return acc + attn_group(b, g)

            x = x + row_sum(lax.fori_loop(0, NG, group, jnp.zeros((8, D), F32)))
            issue_kv(base + jnp.where(l == 0, 36, 50), base + jnp.where(l == 0, 39, 52))
            with _scope("mlp"):
                return mlp(x)

        x = lax.fori_loop(0, 2, layer, jnp.broadcast_to(xf[pl.ds(b, 1), :], (8, D)))
        outf[pl.ds(b, 1), :] = x[0:1, :]
        return done + 1

    done = lax.fori_loop(0, 1 if ONLYTAIL else B - 1, batch_row, 0)

    b = B - 1
    slot = b & 1

    def transpose_k(h0, n=G):
        for i in range(n):
            kt[h0 + i] = _bf16(kbuf[slot, h0 + i]).T.astype(F32)

    pieces = [(range(0, 4), 0, NR), (range(4, 6), 0, NR), (range(6, G), 0, RS), (range(6, G), RS, NR)]

    def chunks(src, dst, heads, sem, lo=0, hi=NR):
        heads = [heads[i] for i in ORDER if i < len(heads)]
        return [(src, dst, b, h, r, sem) for r in ORDER if lo <= r < hi for h in heads]

    queues = (chunks(k32, kbuf, range(h3, h3 + 4), kvsem.at[NG - 1])
              + chunks(v32, vbuf, range(h2, h2 + 2), sem_v2)
              + chunks(v32, vbuf, range(h3 + 2, h3 + 4), sem_piece[0]),
              chunks(v32, vbuf, range(h2 + 2, h2 + 4), sem_v2)
              + chunks(v32, vbuf, range(h3, h3 + 2), sem_piece[0])
              + sum((chunks(v32, vbuf, [h3 + i for i in heads], sem_piece[n], lo, hi)
                     for n, (heads, lo, hi) in enumerate(pieces) if n), []))

    def issue_last(lo, hi):
        for pair in list(zip(*queues))[lo:hi]:
            for queue, args in enumerate(pair):
                chunk(*args).start(priority=queue)

    def wait_piece(n):
        heads, lo, hi = pieces[n]
        wait_all(vbuf.at[slot, pl.ds(h3 + heads[0], len(heads)), pl.ds(lo * 64, (hi - lo) * 64)],
                 sem_piece[n])

    def group(g, acc):
        @pl.when(g == 0)
        def _():
            issue_kv(b * UB + 20 + AHEAD, u_last)
            issue_last(0, VISS[0])

        @pl.when(g == 1)
        def _():
            issue_last(VISS[0], VISS[1])

        hs = pl.ds(g * G, G)
        with _scope("lwait"):
            wait_all(kbuf.at[slot, hs], kvsem.at[g])
            wait_all(vbuf.at[slot, hs], kvsem.at[g])
        with _scope("latt"):
            acc = acc + attn_group(b, g)
            if not NOCOMP:
                transpose_k(g * G)
        return acc

    acc = lax.fori_loop(0, 2, group, jnp.zeros((8, D), F32))
    for i, h in enumerate(MXU_HEADS):
        ktb[i] = pltpu.bitcast(kt[h].astype(BF16), U32)

    @pl.loop(0, 2)
    def _(g):
        for j, hi in enumerate((VISS[2], len(queues[0]))):
            @pl.when(g == j)
            def _():
                issue_last(VISS[1 + j], hi)

        with _scope("kwait"):
            wait_all(kbuf.at[slot, pl.ds(h2 + g * G, G)], kvsem.at[NG - 2 + g])
        with _scope("lscores"):
            if not NOCOMP:
                p, l = scores(b, h2 + g * G)
                p_last[g] = p
                l_last[g] = jnp.broadcast_to(1.0 / l, (8, 128))
                transpose_k(h2 + g * G, TS[0])

    if NOCOMP or STOP:
        wait_all(vbuf.at[slot, pl.ds(h2, G)], sem_v2)
        for n in range(len(pieces)):
            with _scope('piece'):
                wait_piece(n)
        outf[b:b + 1, :] = acc[0:1, :]
        o_ref[...] = outf[...].astype(o_ref.dtype)
        return

    def block(fn, *vals):
        return lax.cond(done > 0, fn, lambda *a: a, *vals)

    def piece_values(n):
        heads, lo, hi = pieces[n]
        wait_piece(n)
        p = p_last[1, :, lo * 128:hi * 128]
        o = None
        for i in heads:
            oi = _dot(p, _bf16(vbuf[slot, h3 + i, lo * 64:hi * 64]))
            o = oi if o is None else jnp.where(row == i, oi, o)
        return o

    def group_out(acc):
        wait_all(vbuf.at[slot, pl.ds(h2, G)], sem_v2)
        o = weighted_values(p_last[0], b, h2, range(G))
        acc = acc + project(o * l_last[0], h2, range(G))
        transpose_k(h2 + TS[0], G - TS[0])
        return (acc,)

    with _scope("pv2"):
        acc, = block(group_out, acc)

    def piece_out(n, acc):
        acc = acc + project(piece_values(n) * l_last[1], h3, pieces[n][0])
        transpose_k(h3 + TS[n], TS[n + 1] - TS[n])
        return (acc,)

    for n in range(2):
        with _scope("pv3"):
            acc, = block(lambda acc: piece_out(n, acc), acc)
    with _scope("pv3c"):
        o, x = block(lambda o, acc: (piece_values(2), xf[b:b + 1, :] + row_sum(acc)),
                     jnp.zeros((8, 128), F32), acc)
    with _scope("pv3d"):
        o = (o + piece_values(3)) * l_last[1]
        heads = pieces[3][0]
        lhs = jnp.concatenate([jnp.broadcast_to(o[i:i + 1], (8, 128)) for i in heads], axis=1)
        r0 = (h3 + heads[0]) * (DH // 2)
        w = jnp.concatenate([_bf16(wo_p[j, r0:r0 + len(heads) * DH // 2]) for j in range(ND)],
                            axis=1)
        x = x + _dot(lhs, w)

    def attention2(x):
        xr = x.astype(BF16).astype(F32)
        xc = _cols(xr, ND)
        mean = jnp.mean(xr, axis=-1, keepdims=True)
        c = xr - mean
        rs = jnp.broadcast_to(lax.rsqrt(jnp.mean(c * c, axis=-1, keepdims=True) + EPS), (8, 128))

        def q_cols(h):
            out = []
            for i in range(0, DH, 8):
                t = [wqt[h, i:i + 8, j * 128:(j + 1) * 128] * xc[j] for j in range(ND)]
                t = (t[0] + t[1]) + (t[2] + t[3]) + t[4]
                out.append(jnp.broadcast_to(jnp.sum(t, axis=1, keepdims=True), (8, 128)))
            return out

        def qk(h, q):
            a = [None] * NR
            for i in range(DH // 8):
                for kb in range(NR):
                    u = kt[h, 8 * i:8 * i + 8, kb * 128:(kb + 1) * 128] * q[i]
                    a[kb] = u if a[kb] is None else a[kb] + u
            for kb in range(NR):
                tr[h, pl.ds(kb, 8, stride=STR), :] = a[kb]
            t = [tr[h, i * STR:i * STR + 8, :] for i in range(8)]
            return ((t[0] + t[1]) + (t[2] + t[3])) + ((t[4] + t[5]) + (t[6] + t[7]))

        def all_reduce(t, lane_op, op):
            for sh in (4, 2, 1):
                t = op(t, pltpu.roll(t, sh, 0))
            return jnp.broadcast_to(lane_op(t, axis=1, keepdims=True), (8, 128))

        def softmax(s):
            p = jnp.exp2((s - all_reduce(s, jnp.max, jnp.maximum)) * rs)
            l = all_reduce(p, jnp.sum, jnp.add)
            r = pltpu.reciprocal(l, approx=True)
            return p, r * (2.0 - l * r)

        def pick(t):
            t = _cols(t, NR)
            o = t[0]
            for kb in range(1, NR):
                o = jnp.where(row == kb, t[kb], o)
            return o

        def pv(h, p):
            return pick(_dot(p, jnp.concatenate(
                [_bf16(vbuf[slot, h, kb * 64:(kb + 1) * 64]) for kb in range(NR)], axis=1)))

        ends, h = {}, 0
        for n in FGROUPS:
            ends[h + n - 1] = range(h, h + n)
            h += n
        assert h == H
        qm, s, pl_, o = {}, {}, {}, {}
        acc = None
        for t in range(H + LAG_F):
            for i, h in enumerate(MXU_HEADS):
                if max(h - LC, 0) == t:
                    qm[h] = _dot(xr, _bf16(wq_p[h]))
            for i, h in enumerate(MXU_HEADS):
                if max(h - LD, 0) == t:
                    s[h] = pick(_dot((qm[h] - mean * csq[i]) * QSCALE, _bf16(ktb[i])))
            if t < H and t not in MXU_HEADS:
                s[t] = qk(t, q_cols(t))
            if 0 <= t - LAG_S < H:
                pl_[t - LAG_S] = softmax(s[t - LAG_S])
            if 0 <= t - LAG_E < H:
                o[t - LAG_E] = pv(t - LAG_E, pl_[t - LAG_E][0]) * pl_[t - LAG_E][1]
            if t - LAG_F in ends:
                hs = ends[t - LAG_F]
                w = jnp.concatenate(
                    [_bf16(wo_p[j, hs[0] * 64:(hs[-1] + 1) * 64]) for j in range(ND)], axis=1)
                u = _dot(jnp.concatenate([o[h] for h in hs], axis=1), w)
                acc = u if acc is None else acc + u
        return x + row_sum(acc)

    if FUSE == 0:
        def last_layer(l, x):
            with _scope("att2"):
                x = lax.cond(l == 1, attention2, lambda x: x, x)
            with _scope("mlp"):
                return mlp(x)

        x = lax.fori_loop(0, 2, last_layer, x)
    else:
        x = mlp(x) if FUSE & 1 else block(lambda x: (mlp(x),), x)[0]
        if FUSE & 2:
            x, = block(lambda x: (mlp(attention2(x)),), x)
        else:
            x, = block(lambda x: (attention2(x),), x)
            x = mlp(x)
    last = lax.broadcasted_iota(jnp.int32, (B, D), 0) == b
    o_ref[...] = jnp.where(last, x, outf[...]).astype(o_ref.dtype)


@jax.jit
def pallas_interleave_layers__sliding_block_cached__mixer_channel_mlp__decode_kernel(
    A_x, A_k_cache, A_v_cache, A_wq, A_wo, B_x, B_w1, B_b1, B_w2, B_b2,
):
    del B_x
    FV = F - FM
    hbm = pl.BlockSpec(memory_space=pltpu.HBM)
    vmem = pltpu.VMEM
    out = pl.pallas_call(
        _kernel,
        out_shape=jax.ShapeDtypeStruct((B, D), A_x.dtype),
        in_specs=[hbm] * 9,
        out_specs=pl.BlockSpec(memory_space=pltpu.VMEM),
        scratch_shapes=[
            vmem((B, D), BF16), vmem((F,), BF16), vmem((D,), BF16),
            vmem((D, H * DH), BF16), vmem((H * DH, D), BF16), vmem((F, D), BF16), vmem((F, D), BF16),
            vmem((B, D), F32), vmem((8, FM), F32), vmem((FM // 128, 8, 128), F32),
            vmem((FV, 128), F32), vmem((8, D), F32),
            vmem((H, D // 2, 128), U32), vmem((ND, H * DH // 2, 128), U32),
            vmem((FM // 128, D // 2, 128), U32), vmem((ND, FM // 2, 128), U32),
            vmem((H, DH, D), F32), vmem((FV, D), F32), vmem((FV, D), F32),
            vmem((2, H, W // 2, DH), U32), vmem((2, H, W // 2, DH), U32),
            vmem((H, DH, W), F32), vmem((len(MXU_HEADS), DH // 2, W), U32), vmem((len(MXU_HEADS), 8, 128), F32),
            vmem((H, 8 * STR, 128), F32), vmem((B * H, DH), F32),
            vmem((2, 8, W), F32), vmem((2, 8, 128), F32), vmem((B, D), F32),
            pltpu.SemaphoreType.DMA((2,)), pltpu.SemaphoreType.DMA((NG,)),
            pltpu.SemaphoreType.DMA((3,)),
        ],
        compiler_params=pltpu.CompilerParams(
            vmem_limit_bytes=120 * 1024 * 1024, disable_bounds_checks=True,
            disable_semaphore_checks=not SEMCHK),
    )(A_x.reshape(B, D), A_k_cache, A_v_cache, A_wq, A_wo, B_w1.T, B_b1, B_w2, B_b2)
    return out.reshape(B, 1, D)
```

```python
import jax
import jax.numpy as jnp
from jax import lax
import jax.experimental.pallas as pl
import jax.experimental.pallas.tpu as pltpu

B, D, H, DH, SK, F = 8, 640, 32, 128, 4096, 1728
W = min(4096, max(256, SK // 4))
EPS = 1e-5
QSCALE = DH ** -0.5 * 1.4426950408889634
F32, BF16, U32 = jnp.float32, jnp.bfloat16, jnp.uint32

G = 8
NG = H // G
ND = D // 128
NR = W // 128

CH = 64
UB = NG * NR
AHEAD = 3
LAST_ISSUE = (10, 32, 52)
RS = 6
TS = 5

FM = 1152
FV = F - FM
MLP_GROUP, MLP_LAG, MLP_LATE = 2, 3, 384

MXU_HEADS = (3, 6)
LAG_S, LAG_PV, LAG_O = 2, 3, 5
O_GROUPS = (4, 4, 4, 4, 4, 4, 2, 2, 2, 1, 1)
STRIDE = 9


def _bf16(words):
    return pltpu.bitcast(words, BF16)


def _words(x):
    return pltpu.bitcast(x, U32)


def _dot(a, b, transposed=False):
    return lax.dot_general(a, b, (((1,), (1 if transposed else 0,)), ((), ())),
                           preferred_element_type=F32)


def _cols(x):
    return [x[:, j:j + 128] for j in range(0, x.shape[1], 128)]


def _hint(i, n):
    return i if isinstance(i, int) else pl.multiple_of(i, n)


def _moments(x):
    def average(t):
        t = _cols(t)
        return jnp.sum((t[0] + t[1]) + (t[2] + t[3]) + t[4], axis=-1, keepdims=True) * (1.0 / D)

    mean = average(x)
    centered = x - mean
    return mean, centered, average(centered * centered)


def _layernorm(x):
    _, centered, var = _moments(x)
    return centered * lax.rsqrt(var + EPS)


def _gelu2(a):
    c = 0.7978845608028654
    return a + a * jnp.tanh(a * (c + (c * 0.044715) * (a * a)))


def _splat(x):
    return jnp.broadcast_to(x, (8, 128))


def _row_sum(x):
    return jnp.broadcast_to(jnp.sum(x, axis=0, keepdims=True), x.shape)


def _kernel(x_hbm, k_hbm, v_hbm, wq_hbm, wo_hbm, w1t_hbm, b1_hbm, w2_hbm, b2_hbm, o_ref,
            x_s, b1_s, b2_s, wq_s, wo_s, w1t_s, w2_s,
            xf, outf, q_all, bias2,
            wq_p, wo_p, w1_p, w2_p, bias1, sum1,
            wqt, w1t_v, w2_v, bias1_v,
            kbuf, vbuf, kt, v_p, kt_p, sumq, tr, p_last, inv_last,
            wsem, ksem, vsem):
    row = lax.broadcasted_iota(jnp.int32, (8, 128), 0)
    last = B - 1
    h2, h3 = H - 2 * G, H - G

    def wait(ref, sem):
        pltpu.make_async_copy(ref, ref, sem).wait()

    def issue_attention_weights(lo, hi):
        @pl.loop(lo, hi)
        def _(i):
            for u in range(5):
                r = pl.ds(pl.multiple_of((u * 16 + (i >> 1)) * 8, 8), 8)
                c = pl.ds(pl.multiple_of((i & 1) * 2048, 2048), 2048)
                pltpu.make_async_copy(wq_hbm.at[r, c], wq_s.at[r, c], wsem.at[1]).start(priority=0)
                if u < 4:
                    r = pl.ds(pl.multiple_of((u * 32 + i) * 32, 32), 32)
                    pltpu.make_async_copy(wo_hbm.at[r], wo_s.at[r], wsem.at[2]).start(priority=1)

    def issue_mlp_weights():
        @pl.loop(0, F // 64)
        def _(i):
            for u in range(2):
                r = pl.ds(pl.multiple_of((u * (F // 64) + i) * 32, 32), 32)
                pltpu.make_async_copy(w1t_hbm.at[r], w1t_s.at[r], wsem.at[3]).start(priority=0)
                pltpu.make_async_copy(w2_hbm.at[r], w2_s.at[r], wsem.at[4]).start(priority=1)

    def chunk(src, dst, b, h, r, sem):
        r0 = _hint(r * CH, CH)
        return pltpu.make_async_copy(src.at[b, pl.ds(h, 2), pl.ds(SK - W + r0, CH)],
                                     dst.at[b & 1, pl.ds(h, 2), pl.ds(r0, CH)], sem)

    u_keys, u_last = B * UB - 2 * NR, B * UB - NR
    pieces = [(range(0, 4), 0, NR), (range(4, 6), 0, NR), (range(6, G), 0, RS), (range(6, G), RS, NR)]
    sem_v2, *sem_piece = [wsem.at[i] for i in range(5)]

    def issue_kv(lo, hi):
        @pl.loop(jnp.minimum(lo, u_last), jnp.minimum(hi, u_last))
        def _(u):
            b = u >> 5
            g = (u >> 3) & (NG - 1)
            steps = [(2 * (u & (NR - 1)) + j, i) for j in range(2) for i in range(0, G, 2)]

            @pl.when(u < u_keys)
            def _():
                for r, i in steps:
                    chunk(k_hbm, kbuf, b, g * G + i, r, ksem.at[g]).start(priority=0)
                    chunk(v_hbm, vbuf, b, g * G + i, r, vsem.at[g]).start(priority=1)

            @pl.when(u >= u_keys)
            def _():
                for r, i in steps:
                    chunk(k_hbm, kbuf, last, h2 + i, r, ksem.at[NG - 2]).start(priority=0)
                    if i < G // 2:
                        c = chunk(k_hbm, kbuf, last, h3 + G // 2 + i, r, ksem.at[NG - 1])
                    else:
                        c = chunk(v_hbm, vbuf, last, h2 + i, r, sem_v2)
                    c.start(priority=1)

    def chunks(src, dst, heads, sem, lo=0, hi=NR):
        return [(src, dst, last, h, r, sem) for r in range(2 * lo, 2 * hi) for h in heads[::2]]

    last_stream = list(zip(
        chunks(k_hbm, kbuf, range(h3, h3 + 4), ksem.at[NG - 1])
        + chunks(v_hbm, vbuf, range(h2, h2 + 2), sem_v2)
        + chunks(v_hbm, vbuf, range(h3 + 2, h3 + 4), sem_piece[0]),
        chunks(v_hbm, vbuf, range(h2 + 2, h2 + 4), sem_v2)
        + chunks(v_hbm, vbuf, range(h3, h3 + 2), sem_piece[0])
        + [c for (heads, lo, hi), sem in zip(pieces[1:], sem_piece[1:])
           for c in chunks(v_hbm, vbuf, [h3 + i for i in heads], sem, lo, hi)],
        strict=True))

    def issue_last(lo, hi):
        for pair in last_stream[lo:hi]:
            for queue, args in enumerate(pair):
                chunk(*args).start(priority=queue)

    small = [pltpu.make_async_copy(src, dst, wsem.at[0])
             for src, dst in ((x_hbm, x_s), (b1_hbm, b1_s), (b2_hbm, b2_s))]
    issue_attention_weights(0, 1)
    for c in small:
        c.start()
    issue_attention_weights(1, 32)
    issue_mlp_weights()
    issue_kv(0, 2)
    for c in small:
        c.wait()
    wait(wq_s, wsem.at[1])
    wait(wo_s, wsem.at[2])

    xf[...] = x_s[...].astype(F32)
    outf[...] = jnp.zeros((B, D), F32)
    b1 = b1_s[...].astype(F32).reshape(1, F)
    bias1[...] = jnp.broadcast_to(b1[:, :FM], (8, FM))
    b1 = jnp.concatenate([b1[:, FM:], jnp.zeros((1, -FV % 128), F32)], axis=1)
    for n in range(0, FV, 128):
        t = jnp.broadcast_to(b1[:, n:n + 128], (128, 128)).T
        bias1_v[n:min(n + 128, FV)] = t[:min(128, FV - n)]
    bias2[...] = jnp.broadcast_to(b2_s[...].astype(F32).reshape(1, D), (8, D))
    y_all = _layernorm(xf[...])

    @pl.loop(0, NG)
    def _(g):
        for i in range(G):
            h = g * G + i
            w = wq_s[:, pl.ds(pl.multiple_of(h * DH, DH), DH)]
            wq_p[h] = _words(w)
            q_all[pl.ds(h, B, stride=H), :] = QSCALE * _dot(y_all, w)
            w = w.T.astype(F32)
            wqt[h] = (w - jnp.mean(w, axis=1, keepdims=True)) * QSCALE
        issue_kv(2 + 2 * g, 4 + 2 * g)

    for i, h in enumerate(MXU_HEADS):
        w = wq_s[:, h * DH:(h + 1) * DH].astype(F32)
        sumq[i] = _splat(jnp.sum(w, axis=0, keepdims=True))

    @pl.loop(0, H)
    def _(h):
        src = pl.ds(pl.multiple_of(h * DH, DH), DH)
        dst = pl.ds(pl.multiple_of(h * (DH // 2), DH // 2), DH // 2)
        for j in range(ND):
            wo_p[j, dst] = _words(wo_s[src, j * 128:(j + 1) * 128])

    issue_kv(10, 12)
    wait(w1t_s, wsem.at[3])
    wait(w2_s, wsem.at[4])
    for n in range(FM // 128):
        w = w1t_s[n * 128:(n + 1) * 128, :].T
        w1_p[n] = _words(w)
        sum1[n] = _splat(jnp.sum(w.astype(F32), axis=0, keepdims=True))
    w = w1t_s[FM:F, :].astype(F32)
    w1t_v[...] = w - jnp.mean(w, axis=1, keepdims=True)
    issue_kv(12, 14)
    for j in range(ND):
        w2_p[j] = _words((0.5 * w2_s[0:FM, j * 128:(j + 1) * 128].astype(F32)).astype(BF16))
    w2_v[...] = 0.5 * w2_s[FM:F, :].astype(F32)
    issue_kv(14, 20 + AHEAD)

    def scores(b, h0):
        q = q_all[pl.ds(_hint(b * H + h0, G), G), :]
        s = None
        for i in range(G):
            t = _cols(_dot(q, kbuf[b & 1, h0 + i], transposed=True))
            s = t if s is None else [jnp.where(row == i, new, old) for new, old in zip(t, s)]
        s = jnp.concatenate(s, axis=1)
        p = jnp.exp2(s - jnp.max(s, axis=-1, keepdims=True))
        return p, jnp.sum(p, axis=-1, keepdims=True)

    def weighted_values(p, b, h0, heads, lo=0, hi=NR, keep=False):
        o = None
        for i in heads:
            v = vbuf[b & 1, h0 + i, lo * 128:hi * 128]
            if keep:
                v_p[h0 + i, lo * 64:hi * 64] = _words(v)
            t = _dot(p, v)
            o = t if o is None else jnp.where(row == i, t, o)
        return o

    def wo_rows(h, n):
        rows = pl.ds(_hint(h * (DH // 2), DH // 2), n * DH // 2)
        return jnp.concatenate([_bf16(wo_p[j, rows]) for j in range(ND)], axis=1)

    def project(o, h0, heads):
        o = jnp.concatenate([jnp.where(row == i, o, 0.0) for i in heads], axis=1)
        return _dot(o, wo_rows(h0 + heads[0], len(heads)))

    def attention_group(b, g, keep=False):
        p, l = scores(b, g * G)
        return project(weighted_values(p, b, g * G, range(G), keep=keep) / l, g * G, range(G))

    def mlp(x):
        xr = x.astype(BF16).astype(F32)
        mean, _, var = _moments(xr)
        scale = _splat(lax.rsqrt(var + EPS * (var + EPS)))
        shift = _splat(mean) * scale

        def up(blocks):
            w = jnp.concatenate([_bf16(w1_p[n]) for n in blocks], axis=1)
            return [_gelu2(t * scale + (bias1[:, n * 128:(n + 1) * 128] - shift * sum1[n]))
                    for t, n in zip(_cols(_dot(xr, w)), blocks)]

        def down(blocks, hidden):
            rows = slice(blocks[0] * 64, (blocks[-1] + 1) * 64)
            w = jnp.concatenate([_bf16(w2_p[j, rows]) for j in range(ND)], axis=1)
            return _dot(jnp.concatenate(hidden, axis=1), w)

        groups = [range(n, min(n + MLP_GROUP, FM // 128)) for n in range(0, FM // 128, MLP_GROUP)]
        hidden, out = [], None
        for t in range(len(groups) + MLP_LAG):
            if t < len(groups):
                hidden.append(up(groups[t]))
            if t >= MLP_LAG:
                u = down(groups[t - MLP_LAG], hidden[t - MLP_LAG])
                out = u if out is None else out + u

        raw = _cols(xr)
        scaled = [t * scale for t in raw]
        acc = [None] * ND
        for i in range(0, FV, 8):
            xs = scaled if i >= MLP_LATE else raw
            t = [w1t_v[i:i + 8, j * 128:(j + 1) * 128] * xs[j] for j in range(ND)]
            t = _splat(jnp.sum((t[0] + t[1]) + (t[2] + t[3]) + t[4], axis=1, keepdims=True))
            t = _gelu2((t if i >= MLP_LATE else t * scale) + bias1_v[i:i + 8])
            for j in range(ND):
                u = w2_v[i:i + 8, j * 128:(j + 1) * 128] * t
                acc[j] = u if acc[j] is None else acc[j] + u
        return (x + bias2[...]) + _row_sum(jnp.concatenate(acc, axis=1)) + out

    @pl.loop(0, last)
    def _(b):
        base = b * UB + AHEAD

        def layer(l, x):
            @pl.when(l == 1)
            def _():
                issue_kv(base + 39, base + 40)
                y = _layernorm(x)
                for g in range(NG):
                    w = jnp.concatenate([_bf16(wq_p[g * G + i]) for i in range(G)], axis=1)
                    t = _cols(_dot(y, w))
                    q = t[0]
                    for i in range(1, G):
                        q = jnp.where(row == i, t[i], q)
                    q_all[pl.ds(pl.multiple_of(b * H + g * G, G), G), :] = q * QSCALE

            def group(g, acc):
                lo = jnp.where(l == 0, 20 + 3 * g, jnp.where(g == 0, 40, 38 + 3 * g))
                hi = jnp.where(l == 0, jnp.where(g == NG - 1, 36, 23 + 3 * g), 41 + 3 * g)
                issue_kv(base + lo, base + hi)

                @pl.when(l == 0)
                def _():
                    wait(kbuf.at[b & 1, pl.ds(g * G, G)], ksem.at[g])
                    wait(vbuf.at[b & 1, pl.ds(g * G, G)], vsem.at[g])

                return acc + attention_group(b, g)

            x = x + _row_sum(lax.fori_loop(0, NG, group, jnp.zeros((8, D), F32)))
            issue_kv(base + jnp.where(l == 0, 36, 50), base + jnp.where(l == 0, 39, 52))
            return mlp(x)

        x = lax.fori_loop(0, 2, layer, jnp.broadcast_to(xf[pl.ds(b, 1), :], (8, D)))
        outf[pl.ds(b, 1), :] = x[0:1, :]

    slot = last & 1

    def transpose_keys(h0, n):
        for i in range(n):
            kt[h0 + i] = kbuf[slot, h0 + i].T.astype(F32)

    def last_group(g, acc):
        @pl.when(g == 0)
        def _():
            issue_kv(last * UB + 20 + AHEAD, u_last)
            issue_last(0, LAST_ISSUE[0])

        @pl.when(g == 1)
        def _():
            issue_last(LAST_ISSUE[0], LAST_ISSUE[1])

        wait(kbuf.at[slot, pl.ds(g * G, G)], ksem.at[g])
        wait(vbuf.at[slot, pl.ds(g * G, G)], vsem.at[g])
        acc = acc + attention_group(last, g, keep=True)
        transpose_keys(g * G, G)
        return acc

    acc = lax.fori_loop(0, 2, last_group, jnp.zeros((8, D), F32))
    for i, h in enumerate(MXU_HEADS):
        kt_p[i] = _words(kt[h].astype(BF16))

    @pl.loop(0, 2)
    def _(g):
        for j, hi in enumerate((LAST_ISSUE[2], len(last_stream))):
            @pl.when(g == j)
            def _():
                issue_last(LAST_ISSUE[1 + j], hi)

        wait(kbuf.at[slot, pl.ds(h2 + g * G, G)], ksem.at[NG - 2 + g])
        p, l = scores(last, h2 + g * G)
        p_last[g] = p
        inv_last[g] = _splat(1.0 / l)
        transpose_keys(h2 + g * G, TS)

    def piece_values(n):
        heads, lo, hi = pieces[n]
        wait(vbuf.at[slot, pl.ds(h3 + heads[0], len(heads)), pl.ds(lo * 128, (hi - lo) * 128)],
             sem_piece[n])
        return weighted_values(p_last[1, :, lo * 128:hi * 128], last, h3, heads, lo, hi, keep=True)

    wait(vbuf.at[slot, pl.ds(h2, G)], sem_v2)
    o = weighted_values(p_last[0], last, h2, range(G), keep=True)
    acc = acc + project(o * inv_last[0], h2, range(G))
    transpose_keys(h2 + TS, G - TS)
    acc = acc + project(piece_values(0) * inv_last[1], h3, pieces[0][0])
    transpose_keys(h3 + TS, G - 1 - TS)
    acc = acc + project(piece_values(1) * inv_last[1], h3, pieces[1][0])
    transpose_keys(H - 1, 1)
    o = piece_values(2)
    x = xf[last:B, :] + _row_sum(acc)
    o = (o + piece_values(3)) * inv_last[1]
    heads = pieces[3][0]
    x = x + _dot(jnp.concatenate([_splat(o[i:i + 1]) for i in heads], axis=1),
                 wo_rows(h3 + heads[0], len(heads)))

    def second_attention(x):
        xr = x.astype(BF16).astype(F32)
        xs = _cols(xr)
        mean, _, var = _moments(xr)
        scale = _splat(lax.rsqrt(var + EPS))

        def query(h):
            q = []
            for i in range(0, DH, 8):
                t = [wqt[h, i:i + 8, j * 128:(j + 1) * 128] * xs[j] for j in range(ND)]
                t = ((t[0] + t[1]) + t[2]) + (t[3] + t[4])
                q.append(_splat(jnp.sum(t, axis=1, keepdims=True)))
            return q

        def head_scores(h, q):
            a = [None] * NR
            for i in range(DH // 8):
                for kb in range(NR):
                    u = kt[h, 8 * i:8 * i + 8, kb * 128:(kb + 1) * 128] * q[i]
                    a[kb] = u if a[kb] is None else a[kb] + u
            for kb in range(NR):
                tr[h, pl.ds(kb, 8, stride=STRIDE), :] = a[kb]
            t = [tr[h, i * STRIDE:i * STRIDE + 8, :] for i in range(8)]
            return ((t[0] + t[1]) + (t[2] + t[3])) + ((t[4] + t[5]) + (t[6] + t[7]))

        def diagonal(t):
            t = _cols(t)
            o = t[0]
            for kb in range(1, NR):
                o = jnp.where(row == kb, t[kb], o)
            return o

        def all_reduce(t, op, lane_op):
            for shift in (4, 2, 1):
                t = op(t, pltpu.roll(t, shift, 0))
            return _splat(lane_op(t, axis=1, keepdims=True))

        def softmax(s):
            p = jnp.exp2((s - all_reduce(s, jnp.maximum, jnp.max)) * scale)
            l = all_reduce(p, jnp.add, jnp.sum)
            r = pltpu.reciprocal(l, approx=True)
            return p, r * (2.0 - l * r)

        ends, h = {}, 0
        for n in O_GROUPS:
            ends[h + n - 1] = range(h, h + n)
            h += n
        s = {h: _dot(xr, _bf16(wq_p[h])) for h in MXU_HEADS}
        for i, h in enumerate(MXU_HEADS):
            s[h] = diagonal(_dot((s[h] - mean * sumq[i]) * QSCALE, _bf16(kt_p[i])))
        p, o, acc = {}, {}, None
        for t in range(H + LAG_O):
            if t < H and t not in MXU_HEADS:
                s[t] = head_scores(t, query(t))
            if 0 <= t - LAG_S < H:
                p[t - LAG_S] = softmax(s[t - LAG_S])
            if 0 <= t - LAG_PV < H:
                h = t - LAG_PV
                v = jnp.concatenate(
                    [_bf16(v_p[h, kb * 64:(kb + 1) * 64]) for kb in range(NR)], axis=1)
                o[h] = diagonal(_dot(p[h][0], v)) * p[h][1]
            if t - LAG_O in ends:
                heads = ends[t - LAG_O]
                u = _dot(jnp.concatenate([o[h] for h in heads], axis=1),
                         wo_rows(heads[0], len(heads)))
                acc = u if acc is None else acc + u
        return x + _row_sum(acc)

    def last_layer(l, x):
        return mlp(lax.cond(l == 1, second_attention, lambda x: x, x))

    x = lax.fori_loop(0, 2, last_layer, x)
    is_last = lax.broadcasted_iota(jnp.int32, (B, D), 0) == last
    o_ref[...] = jnp.where(is_last, x, outf[...]).astype(o_ref.dtype)


@jax.jit
def pallas_interleave_layers__sliding_block_cached__mixer_channel_mlp__decode_kernel(
    A_x: jax.Array,
    A_k_cache: jax.Array,
    A_v_cache: jax.Array,
    A_wq: jax.Array,
    A_wo: jax.Array,
    B_x: jax.Array,
    B_w1: jax.Array,
    B_b1: jax.Array,
    B_w2: jax.Array,
    B_b2: jax.Array,
):
    del B_x
    vmem = pltpu.VMEM
    out = pl.pallas_call(
        _kernel,
        out_shape=jax.ShapeDtypeStruct((B, D), A_x.dtype),
        in_specs=[pl.BlockSpec(memory_space=pltpu.HBM)] * 9,
        out_specs=pl.BlockSpec(memory_space=pltpu.VMEM),
        scratch_shapes=[
            vmem((B, D), BF16), vmem((F,), BF16), vmem((D,), BF16),
            vmem((D, H * DH), BF16), vmem((H * DH, D), BF16), vmem((F, D), BF16), vmem((F, D), BF16),
            vmem((B, D), F32), vmem((B, D), F32), vmem(((B + 1) * H, DH), F32), vmem((8, D), F32),
            vmem((H, D // 2, 128), U32), vmem((ND, H * DH // 2, 128), U32),
            vmem((FM // 128, D // 2, 128), U32), vmem((ND, FM // 2, 128), U32),
            vmem((8, FM), F32), vmem((FM // 128, 8, 128), F32),
            vmem((H, DH, D), F32), vmem((FV, D), F32), vmem((FV, D), F32), vmem((FV, 128), F32),
            vmem((2, H, W, DH), BF16), vmem((2, H, W, DH), BF16),
            vmem((H, DH, W), F32), vmem((H, W // 2, DH), U32),
            vmem((len(MXU_HEADS), DH // 2, W), U32), vmem((len(MXU_HEADS), 8, 128), F32),
            vmem((H, 8 * (STRIDE + 1), 128), F32), vmem((2, 8, W), F32), vmem((2, 8, 128), F32),
            pltpu.SemaphoreType.DMA((5,)), pltpu.SemaphoreType.DMA((NG,)),
            pltpu.SemaphoreType.DMA((NG,)),
        ],
        compiler_params=pltpu.CompilerParams(
            vmem_limit_bytes=120 * 1024 * 1024,
            disable_bounds_checks=True,
            disable_semaphore_checks=True,
        ),
    )(A_x.reshape(B, D), A_k_cache, A_v_cache, A_wq, A_wo, B_w1.T, B_b1, B_w2, B_b2)
    return out.reshape(B, 1, D)
```

```python
import jax
import jax.numpy as jnp
from jax import lax
import jax.experimental.pallas as pl
import jax.experimental.pallas.tpu as pltpu

B, D, H, DH, SK, F = 8, 640, 32, 128, 4096, 1728
W = min(4096, max(256, SK // 4))
EPS = 1e-5
QSCALE = DH ** -0.5 * 1.4426950408889634
F32, BF16, U32 = jnp.float32, jnp.bfloat16, jnp.uint32

G = 8
NG = H // G
ND = D // 128
NR = W // 128

CH = 64
UB = NG * NR
AHEAD = 3
LAST_ISSUE = (10, 32, 52)
RS = 6
TS = 5

FM = 1152
FV = F - FM
MLP_GROUP, MLP_LAG, MLP_LATE = 2, 3, 384

EARLY, LATE = (2, 10), (0, 1, 8)
ORDER = (3, 4, 2, 5, 6, 7) + tuple(range(9, H))
LAG_S, LAG_PV, LAG_O = 2, 3, 5
O_GROUPS = (1, 4, 4, 4, 4, 4, 4, 2, 1, 1)
STRIDE = 9


def _bf16(words):
    return pltpu.bitcast(words, BF16)


def _words(x):
    return pltpu.bitcast(x, U32)


def _dot(a, b, transposed=False):
    return lax.dot_general(a, b, (((1,), (1 if transposed else 0,)), ((), ())),
                           preferred_element_type=F32)


def _cols(x):
    return [x[:, j:j + 128] for j in range(0, x.shape[1], 128)]


def _hint(i, n):
    return i if isinstance(i, int) else pl.multiple_of(i, n)


def _moments(x):
    def average(t):
        t = _cols(t)
        return jnp.sum((t[0] + t[1]) + (t[2] + t[3]) + t[4], axis=-1, keepdims=True) * (1.0 / D)

    mean = average(x)
    centered = x - mean
    return mean, centered, average(centered * centered)


def _layernorm(x):
    _, centered, var = _moments(x)
    return centered * lax.rsqrt(var + EPS)


def _gelu2(a):
    c = 0.7978845608028654
    return a + a * jnp.tanh(a * (c + (c * 0.044715) * (a * a)))


def _splat(x):
    return jnp.broadcast_to(x, (8, 128))


def _row_sum(x):
    return jnp.broadcast_to(jnp.sum(x, axis=0, keepdims=True), x.shape)


def _kernel(x_hbm, k_hbm, v_hbm, wq_hbm, wo_hbm, w1t_hbm, b1_hbm, w2_hbm, b2_hbm, o_ref,
            x_s, b1_s, b2_s, wq_s, wo_s, w1t_s, w2_s,
            xf, outf, q_all, bias2,
            wq_p, wo_p, w1_p, w2_p, bias1, sum1,
            wqt, wo_v, w1t_v, w2_v, bias1_v,
            kbuf, vbuf, kt, v_p, kt_p, vt, sumq, tr, p_last, inv_last,
            wsem, ksem, vsem):
    row = lax.broadcasted_iota(jnp.int32, (8, 128), 0)
    last = B - 1
    h2, h3 = H - 2 * G, H - G

    def wait(ref, sem):
        pltpu.make_async_copy(ref, ref, sem).wait()

    def issue_attention_weights(lo, hi):
        @pl.loop(lo, hi)
        def _(i):
            for u in range(5):
                r = pl.ds(pl.multiple_of((u * 16 + (i >> 1)) * 8, 8), 8)
                c = pl.ds(pl.multiple_of((i & 1) * 2048, 2048), 2048)
                pltpu.make_async_copy(wq_hbm.at[r, c], wq_s.at[r, c], wsem.at[1]).start(priority=0)
                if u < 4:
                    r = pl.ds(pl.multiple_of((u * 32 + i) * 32, 32), 32)
                    pltpu.make_async_copy(wo_hbm.at[r], wo_s.at[r], wsem.at[2]).start(priority=1)

    def issue_mlp_weights():
        @pl.loop(0, F // 64)
        def _(i):
            for u in range(2):
                r = pl.ds(pl.multiple_of((u * (F // 64) + i) * 32, 32), 32)
                pltpu.make_async_copy(w1t_hbm.at[r], w1t_s.at[r], wsem.at[3]).start(priority=0)
                pltpu.make_async_copy(w2_hbm.at[r], w2_s.at[r], wsem.at[4]).start(priority=1)

    def chunk(src, dst, b, h, r, sem):
        r0 = _hint(r * CH, CH)
        return pltpu.make_async_copy(src.at[b, pl.ds(h, 2), pl.ds(SK - W + r0, CH)],
                                     dst.at[b & 1, pl.ds(h, 2), pl.ds(r0, CH)], sem)

    u_keys, u_last = B * UB - 2 * NR, B * UB - NR
    pieces = [(range(0, 4), 0, NR), (range(4, 6), 0, NR), (range(6, G), 0, RS), (range(6, G), RS, NR)]
    sem_v2, *sem_piece = [wsem.at[i] for i in range(5)]

    def issue_kv(lo, hi):
        @pl.loop(jnp.minimum(lo, u_last), jnp.minimum(hi, u_last))
        def _(u):
            b = u >> 5
            g = (u >> 3) & (NG - 1)
            steps = [(2 * (u & (NR - 1)) + j, i) for j in range(2) for i in range(0, G, 2)]

            @pl.when(u < u_keys)
            def _():
                for r, i in steps:
                    chunk(k_hbm, kbuf, b, g * G + i, r, ksem.at[g]).start(priority=0)
                    chunk(v_hbm, vbuf, b, g * G + i, r, vsem.at[g]).start(priority=1)

            @pl.when(u >= u_keys)
            def _():
                for r, i in steps:
                    chunk(k_hbm, kbuf, last, h2 + i, r, ksem.at[NG - 2]).start(priority=0)
                    if i < G // 2:
                        c = chunk(k_hbm, kbuf, last, h3 + G // 2 + i, r, ksem.at[NG - 1])
                    else:
                        c = chunk(v_hbm, vbuf, last, h2 + i, r, sem_v2)
                    c.start(priority=1)

    def chunks(src, dst, heads, sem, lo=0, hi=NR):
        return [(src, dst, last, h, r, sem) for r in range(2 * lo, 2 * hi) for h in heads[::2]]

    last_stream = list(zip(
        chunks(k_hbm, kbuf, range(h3, h3 + 4), ksem.at[NG - 1])
        + chunks(v_hbm, vbuf, range(h2, h2 + 2), sem_v2)
        + chunks(v_hbm, vbuf, range(h3 + 2, h3 + 4), sem_piece[0]),
        chunks(v_hbm, vbuf, range(h2 + 2, h2 + 4), sem_v2)
        + chunks(v_hbm, vbuf, range(h3, h3 + 2), sem_piece[0])
        + [c for (heads, lo, hi), sem in zip(pieces[1:], sem_piece[1:])
           for c in chunks(v_hbm, vbuf, [h3 + i for i in heads], sem, lo, hi)],
        strict=True))

    def issue_last(lo, hi):
        for pair in last_stream[lo:hi]:
            for queue, args in enumerate(pair):
                chunk(*args).start(priority=queue)

    small = [pltpu.make_async_copy(src, dst, wsem.at[0])
             for src, dst in ((x_hbm, x_s), (b1_hbm, b1_s), (b2_hbm, b2_s))]
    issue_attention_weights(0, 1)
    for c in small:
        c.start()
    issue_attention_weights(1, 32)
    issue_mlp_weights()
    issue_kv(0, 2)
    for c in small:
        c.wait()
    wait(wq_s, wsem.at[1])
    wait(wo_s, wsem.at[2])

    xf[...] = x_s[...].astype(F32)
    outf[...] = jnp.zeros((B, D), F32)
    b1 = b1_s[...].astype(F32).reshape(1, F)
    bias1[...] = jnp.broadcast_to(b1[:, :FM], (8, FM))
    b1 = jnp.concatenate([b1[:, FM:], jnp.zeros((1, -FV % 128), F32)], axis=1)
    for n in range(0, FV, 128):
        t = jnp.broadcast_to(b1[:, n:n + 128], (128, 128)).T
        bias1_v[n:min(n + 128, FV)] = t[:min(128, FV - n)]
    bias2[...] = jnp.broadcast_to(b2_s[...].astype(F32).reshape(1, D), (8, D))
    y_all = _layernorm(xf[...])

    @pl.loop(0, NG)
    def _(g):
        for i in range(G):
            h = g * G + i
            w = wq_s[:, pl.ds(pl.multiple_of(h * DH, DH), DH)]
            wq_p[h] = _words(w)
            q_all[pl.ds(h, B, stride=H), :] = QSCALE * _dot(y_all, w)
            w = w.T.astype(F32)
            wqt[h] = (w - jnp.mean(w, axis=1, keepdims=True)) * QSCALE
        issue_kv(2 + 2 * g, 4 + 2 * g)

    for i, h in enumerate(EARLY + LATE):
        w = wq_s[:, h * DH:(h + 1) * DH].astype(F32)
        sumq[i] = _splat(jnp.sum(w, axis=0, keepdims=True))
    for i, h in enumerate(LATE):
        wo_v[i] = wo_s[h * DH:(h + 1) * DH, :].astype(F32)

    @pl.loop(0, H)
    def _(h):
        src = pl.ds(pl.multiple_of(h * DH, DH), DH)
        dst = pl.ds(pl.multiple_of(h * (DH // 2), DH // 2), DH // 2)
        for j in range(ND):
            wo_p[j, dst] = _words(wo_s[src, j * 128:(j + 1) * 128])

    issue_kv(10, 12)
    wait(w1t_s, wsem.at[3])
    wait(w2_s, wsem.at[4])
    for n in range(FM // 128):
        w = w1t_s[n * 128:(n + 1) * 128, :].T
        w1_p[n] = _words(w)
        sum1[n] = _splat(jnp.sum(w.astype(F32), axis=0, keepdims=True))
    w = w1t_s[FM:F, :].astype(F32)
    w1t_v[...] = w - jnp.mean(w, axis=1, keepdims=True)
    issue_kv(12, 14)
    for j in range(ND):
        w2_p[j] = _words((0.5 * w2_s[0:FM, j * 128:(j + 1) * 128].astype(F32)).astype(BF16))
    w2_v[...] = 0.5 * w2_s[FM:F, :].astype(F32)
    issue_kv(14, 20 + AHEAD)

    def scores(b, h0):
        q = q_all[pl.ds(_hint(b * H + h0, G), G), :]
        s = None
        for i in range(G):
            t = _cols(_dot(q, kbuf[b & 1, h0 + i], transposed=True))
            s = t if s is None else [jnp.where(row == i, new, old) for new, old in zip(t, s)]
        s = jnp.concatenate(s, axis=1)
        p = jnp.exp2(s - jnp.max(s, axis=-1, keepdims=True))
        return p, jnp.sum(p, axis=-1, keepdims=True)

    def weighted_values(p, b, h0, heads, lo=0, hi=NR, keep=False):
        o = None
        for i in heads:
            v = vbuf[b & 1, h0 + i, lo * 128:hi * 128]
            if keep:
                v_p[h0 + i, lo * 64:hi * 64] = _words(v)
            t = _dot(p, v)
            o = t if o is None else jnp.where(row == i, t, o)
        return o

    def wo_rows(h, n):
        rows = pl.ds(_hint(h * (DH // 2), DH // 2), n * DH // 2)
        return jnp.concatenate([_bf16(wo_p[j, rows]) for j in range(ND)], axis=1)

    def project(o, h0, heads):
        o = jnp.concatenate([jnp.where(row == i, o, 0.0) for i in heads], axis=1)
        return _dot(o, wo_rows(h0 + heads[0], len(heads)))

    def attention_group(b, g, keep=False):
        p, l = scores(b, g * G)
        return project(weighted_values(p, b, g * G, range(G), keep=keep) / l, g * G, range(G))

    def mlp(x):
        xr = x.astype(BF16).astype(F32)
        mean, _, var = _moments(xr)
        scale = _splat(lax.rsqrt(var + EPS * (var + EPS)))
        shift = _splat(mean) * scale

        def up(blocks):
            w = jnp.concatenate([_bf16(w1_p[n]) for n in blocks], axis=1)
            return [_gelu2(t * scale + (bias1[:, n * 128:(n + 1) * 128] - shift * sum1[n]))
                    for t, n in zip(_cols(_dot(xr, w)), blocks)]

        def down(blocks, hidden):
            rows = slice(blocks[0] * 64, (blocks[-1] + 1) * 64)
            w = jnp.concatenate([_bf16(w2_p[j, rows]) for j in range(ND)], axis=1)
            return _dot(jnp.concatenate(hidden, axis=1), w)

        groups = [range(n, min(n + MLP_GROUP, FM // 128)) for n in range(0, FM // 128, MLP_GROUP)]
        hidden, out = [], None
        for t in range(len(groups) + MLP_LAG):
            if t < len(groups):
                hidden.append(up(groups[t]))
            if t >= MLP_LAG:
                u = down(groups[t - MLP_LAG], hidden[t - MLP_LAG])
                out = u if out is None else out + u

        raw = _cols(xr)
        scaled = [t * scale for t in raw]
        acc = [None] * ND
        for i in range(0, FV, 8):
            xs = scaled if i >= MLP_LATE else raw
            t = [w1t_v[i:i + 8, j * 128:(j + 1) * 128] * xs[j] for j in range(ND)]
            t = _splat(jnp.sum((t[0] + t[1]) + (t[2] + t[3]) + t[4], axis=1, keepdims=True))
            t = _gelu2((t if i >= MLP_LATE else t * scale) + bias1_v[i:i + 8])
            for j in range(ND):
                u = w2_v[i:i + 8, j * 128:(j + 1) * 128] * t
                acc[j] = u if acc[j] is None else acc[j] + u
        return (x + bias2[...]) + _row_sum(jnp.concatenate(acc, axis=1)) + out

    @pl.loop(0, last)
    def _(b):
        base = b * UB + AHEAD

        def layer(l, x):
            @pl.when(l == 1)
            def _():
                issue_kv(base + 39, base + 40)
                y = _layernorm(x)
                for g in range(NG):
                    w = jnp.concatenate([_bf16(wq_p[g * G + i]) for i in range(G)], axis=1)
                    t = _cols(_dot(y, w))
                    q = t[0]
                    for i in range(1, G):
                        q = jnp.where(row == i, t[i], q)
                    q_all[pl.ds(pl.multiple_of(b * H + g * G, G), G), :] = q * QSCALE

            def group(g, acc):
                lo = jnp.where(l == 0, 20 + 3 * g, jnp.where(g == 0, 40, 38 + 3 * g))
                hi = jnp.where(l == 0, jnp.where(g == NG - 1, 36, 23 + 3 * g), 41 + 3 * g)
                issue_kv(base + lo, base + hi)

                @pl.when(l == 0)
                def _():
                    wait(kbuf.at[b & 1, pl.ds(g * G, G)], ksem.at[g])
                    wait(vbuf.at[b & 1, pl.ds(g * G, G)], vsem.at[g])

                return acc + attention_group(b, g)

            x = x + _row_sum(lax.fori_loop(0, NG, group, jnp.zeros((8, D), F32)))
            issue_kv(base + jnp.where(l == 0, 36, 50), base + jnp.where(l == 0, 39, 52))
            return mlp(x)

        x = lax.fori_loop(0, 2, layer, jnp.broadcast_to(xf[pl.ds(b, 1), :], (8, D)))
        outf[pl.ds(b, 1), :] = x[0:1, :]

    slot = last & 1

    def transpose_keys(h0, n):
        for i in range(n):
            kt[h0 + i] = kbuf[slot, h0 + i].T.astype(F32)

    def last_group(g, acc):
        @pl.when(g == 0)
        def _():
            issue_kv(last * UB + 20 + AHEAD, u_last)
            issue_last(0, LAST_ISSUE[0])

        @pl.when(g == 1)
        def _():
            issue_last(LAST_ISSUE[0], LAST_ISSUE[1])

        wait(kbuf.at[slot, pl.ds(g * G, G)], ksem.at[g])
        wait(vbuf.at[slot, pl.ds(g * G, G)], vsem.at[g])
        acc = acc + attention_group(last, g, keep=True)
        for i in range(G):
            t = kbuf[slot, g * G + i].T
            kt[g * G + i] = t.astype(F32)
            if i < 3:
                kt_p[g, i] = _words(t)
            if i < 2:
                vt[g, i] = vbuf[slot, g * G + i].T.astype(F32)
        return acc

    acc = lax.fori_loop(0, 2, last_group, jnp.zeros((8, D), F32))

    @pl.loop(0, 2)
    def _(g):
        for j, hi in enumerate((LAST_ISSUE[2], len(last_stream))):
            @pl.when(g == j)
            def _():
                issue_last(LAST_ISSUE[1 + j], hi)

        wait(kbuf.at[slot, pl.ds(h2 + g * G, G)], ksem.at[NG - 2 + g])
        p, l = scores(last, h2 + g * G)
        p_last[g] = p
        inv_last[g] = _splat(1.0 / l)
        transpose_keys(h2 + g * G, TS)

    def piece_values(n):
        heads, lo, hi = pieces[n]
        wait(vbuf.at[slot, pl.ds(h3 + heads[0], len(heads)), pl.ds(lo * 128, (hi - lo) * 128)],
             sem_piece[n])
        return weighted_values(p_last[1, :, lo * 128:hi * 128], last, h3, heads, lo, hi, keep=True)

    wait(vbuf.at[slot, pl.ds(h2, G)], sem_v2)
    o = weighted_values(p_last[0], last, h2, range(G), keep=True)
    acc = acc + project(o * inv_last[0], h2, range(G))
    transpose_keys(h2 + TS, G - TS)
    acc = acc + project(piece_values(0) * inv_last[1], h3, pieces[0][0])
    transpose_keys(h3 + TS, G - 1 - TS)
    acc = acc + project(piece_values(1) * inv_last[1], h3, pieces[1][0])
    transpose_keys(H - 1, 1)
    o = piece_values(2)
    x = xf[last:B, :] + _row_sum(acc)
    o = (o + piece_values(3)) * inv_last[1]
    heads = pieces[3][0]
    x = x + _dot(jnp.concatenate([_splat(o[i:i + 1]) for i in heads], axis=1),
                 wo_rows(h3 + heads[0], len(heads)))

    def second_attention(x):
        xr = x.astype(BF16).astype(F32)
        xs = _cols(xr)
        mean, _, var = _moments(xr)
        scale = _splat(lax.rsqrt(var + EPS))

        def query(h):
            q = []
            for i in range(0, DH, 8):
                t = [wqt[h, i:i + 8, j * 128:(j + 1) * 128] * xs[j] for j in range(ND)]
                t = (t[0] + t[1]) + ((t[2] + t[3]) + t[4])
                q.append(_splat(jnp.sum(t, axis=1, keepdims=True)))
            return q

        def head_scores(h, q):
            a = [None] * NR
            for i in range(DH // 8):
                for kb in reversed(range(NR)):
                    u = kt[h, 8 * i:8 * i + 8, kb * 128:(kb + 1) * 128] * q[i]
                    a[kb] = u if a[kb] is None else a[kb] + u
            for kb in reversed(range(NR)):
                tr[h, pl.ds(kb, 8, stride=STRIDE), :] = a[kb]
            t = [tr[h, i * STRIDE:i * STRIDE + 8, :] for i in range(8)]
            return ((t[0] + t[1]) + (t[2] + t[3])) + ((t[4] + t[5]) + (t[6] + t[7]))

        def diagonal(t):
            t = _cols(t)
            o = t[0]
            for kb in range(1, NR):
                o = jnp.where(row == kb, t[kb], o)
            return o

        def all_reduce(t, op, lane_op):
            for shift in (4, 2, 1):
                t = op(t, pltpu.roll(t, shift, 0))
            return _splat(lane_op(t, axis=1, keepdims=True))

        def softmax(s):
            p = jnp.exp2((s - all_reduce(s, jnp.maximum, jnp.max)) * scale)
            l = all_reduce(p, jnp.add, jnp.sum)
            r = pltpu.reciprocal(l, approx=True)
            return p, r * (2.0 - l * r)

        ends, t = {}, 0
        for n in O_GROUPS:
            ends[t + n - 1] = ORDER[t:t + n]
            t += n
        s = {h: _dot(xr, _bf16(wq_p[h])) for h in EARLY + LATE}
        for i, h in enumerate(EARLY + LATE):
            q = (s[h] - mean * sumq[i]) * QSCALE
            s[h] = diagonal(_dot(q, _bf16(kt_p[h // G, h % G])))
        p, o, acc = {}, {}, None
        for t in range(len(ORDER) + LAG_O):
            if t < len(ORDER) and ORDER[t] not in EARLY:
                s[ORDER[t]] = head_scores(ORDER[t], query(ORDER[t]))
            if 0 <= t - LAG_S < len(ORDER):
                p[ORDER[t - LAG_S]] = softmax(s[ORDER[t - LAG_S]])
            if 0 <= t - LAG_PV < len(ORDER):
                h = ORDER[t - LAG_PV]
                v = jnp.concatenate(
                    [_bf16(v_p[h, kb * 64:(kb + 1) * 64]) for kb in range(NR)], axis=1)
                o[h] = diagonal(_dot(p[h][0], v)) * p[h][1]
            if t - LAG_O in ends:
                heads = ends[t - LAG_O]
                u = _dot(jnp.concatenate([o[h] for h in heads], axis=1),
                         jnp.concatenate([wo_rows(h, 1) for h in heads], axis=0))
                acc = u if acc is None else acc + u
        late = [None] * ND
        for n, h in enumerate(LATE):
            ph, inv = softmax(s[h])
            ph = ph * inv
            ph = [_splat(ph[kb:kb + 1]) for kb in range(NR)]
            for i in range(0, DH, 8):
                t = [vt[h // G, h % G, i:i + 8, kb * 128:(kb + 1) * 128] * ph[kb] for kb in range(NR)]
                t = ((t[0] + t[1]) + (t[2] + t[3])) + ((t[4] + t[5]) + (t[6] + t[7]))
                t = _splat(jnp.sum(t, axis=1, keepdims=True))
                for j in range(ND):
                    u = wo_v[n, i:i + 8, j * 128:(j + 1) * 128] * t
                    late[j] = u if late[j] is None else late[j] + u
        return x + _row_sum(acc + jnp.concatenate(late, axis=1))

    def last_layer(l, x):
        return mlp(lax.cond(l == 1, second_attention, lambda x: x, x))

    x = lax.fori_loop(0, 2, last_layer, x)
    is_last = lax.broadcasted_iota(jnp.int32, (B, D), 0) == last
    o_ref[...] = jnp.where(is_last, x, outf[...]).astype(o_ref.dtype)


@jax.jit
def pallas_interleave_layers__sliding_block_cached__mixer_channel_mlp__decode_kernel(
    A_x: jax.Array,
    A_k_cache: jax.Array,
    A_v_cache: jax.Array,
    A_wq: jax.Array,
    A_wo: jax.Array,
    B_x: jax.Array,
    B_w1: jax.Array,
    B_b1: jax.Array,
    B_w2: jax.Array,
    B_b2: jax.Array,
):
    del B_x
    vmem = pltpu.VMEM
    out = pl.pallas_call(
        _kernel,
        out_shape=jax.ShapeDtypeStruct((B, D), A_x.dtype),
        in_specs=[pl.BlockSpec(memory_space=pltpu.HBM)] * 9,
        out_specs=pl.BlockSpec(memory_space=pltpu.VMEM),
        scratch_shapes=[
            vmem((B, D), BF16), vmem((F,), BF16), vmem((D,), BF16),
            vmem((D, H * DH), BF16), vmem((H * DH, D), BF16), vmem((F, D), BF16), vmem((F, D), BF16),
            vmem((B, D), F32), vmem((B, D), F32), vmem(((B + 1) * H, DH), F32), vmem((8, D), F32),
            vmem((H, D // 2, 128), U32), vmem((ND, H * DH // 2, 128), U32),
            vmem((FM // 128, D // 2, 128), U32), vmem((ND, FM // 2, 128), U32),
            vmem((8, FM), F32), vmem((FM // 128, 8, 128), F32),
            vmem((H, DH, D), F32), vmem((len(LATE), DH, D), F32),
            vmem((FV, D), F32), vmem((FV, D), F32), vmem((FV, 128), F32),
            vmem((2, H, W, DH), BF16), vmem((2, H, W, DH), BF16),
            vmem((H, DH, W), F32), vmem((H, W // 2, DH), U32),
            vmem((2, 3, DH // 2, W), U32), vmem((2, 2, DH, W), F32),
            vmem((len(EARLY + LATE), 8, 128), F32),
            vmem((H, 8 * (STRIDE + 1), 128), F32), vmem((2, 8, W), F32), vmem((2, 8, 128), F32),
            pltpu.SemaphoreType.DMA((5,)), pltpu.SemaphoreType.DMA((NG,)),
            pltpu.SemaphoreType.DMA((NG,)),
        ],
        compiler_params=pltpu.CompilerParams(
            vmem_limit_bytes=120 * 1024 * 1024,
            disable_bounds_checks=True,
            disable_semaphore_checks=True,
        ),
    )(A_x.reshape(B, D), A_k_cache, A_v_cache, A_wq, A_wo, B_w1.T, B_b1, B_w2, B_b2)
    return out.reshape(B, 1, D)
```
